```python
import jax
import jax.numpy as jnp

def _softmax(x, axis=-1):
    return jax.nn.softmax(x, axis=axis)
def _gelu(x):
    return jax.nn.gelu(x, approximate=True)
def _silu(x):
    return jax.nn.silu(x)
def _sigmoid(x):
    return jax.nn.sigmoid(x)
def _layernorm(x, axis=-1, eps=1e-5):
    m = jnp.mean(x, axis=axis, keepdims=True)
    v = jnp.var(x, axis=axis, keepdims=True)
    return (x - m) / jnp.sqrt(v + eps)
def _scatter_add(tgt, idx, src, axis=0):
    return tgt.at[idx].add(src)
def _segment_sum(src, seg, n):
    return jax.ops.segment_sum(src, seg, n)
class _Rng:
    def __init__(self, key):
        self._k = key
    def _next(self):
        self._k, sub = jax.random.split(self._k)
        return sub
    def normal(self, shape):
        return jax.random.normal(self._next(), shape, dtype=jnp.bfloat16)
    def randint(self, lo, hi, shape):
        return jax.random.randint(self._next(), shape, lo, hi, dtype=jnp.int32)
    def uniform(self, shape, lo=0.0, hi=1.0):
        return jax.random.uniform(self._next(), shape, jnp.bfloat16, lo, hi)
    def permutation(self, n):
        return jax.random.permutation(self._next(), n)


kernel_name = 'recurrent_scan__sliding_block_cached__moe_arch_mod__prompt'

def setup_inputs():
    _rng = _Rng(jax.random.key(int.from_bytes(__import__("os").urandom(4), "little")))
    _w = (lambda a: (lambda t: t.astype(jnp.bfloat16) if jnp.issubdtype(t.dtype, jnp.floating) else t)(jnp.asarray(a)))
    def _A_setup():
        B, Sq, D = 1, 2048, 640
        Hq, Hkv, Sk, Dh = 32, 32, 2048, 192
        assert Hq % Hkv == 0, (Hq, Hkv)
        return {
            "x": _w((lambda *s: _rng.normal(s) * 0.05)(B, Sq, D)),
            "k_cache": _w((lambda *s: _rng.normal(s) * 0.05)(B, Hkv, Sk, Dh)),
            "v_cache": _w((lambda *s: _rng.normal(s) * 0.05)(B, Hkv, Sk, Dh)),
            "wq": _w((lambda *s: _rng.normal(s) * 0.05)(D, Hq * Dh) * (D ** -0.5)),
            "wo": _w((lambda *s: _rng.normal(s) * 0.05)(Hq * Dh, D) * ((Hq * Dh) ** -0.5)),
        }
    _A_in = _A_setup()

    def _B_setup():
        B, S, D, F, C = 1, 2048, 640, 1536, 2
        return {
            "x": _w((lambda *s: _rng.normal(s) * 0.05)(B, S, D)),
            "w_r": _w((lambda *s: _rng.normal(s) * 0.05)(D)),
            "w_gate": _w((lambda *s: _rng.normal(s) * 0.05)(D, F)),
            "w_up": _w((lambda *s: _rng.normal(s) * 0.05)(D, F)),
            "w_down": _w((lambda *s: _rng.normal(s) * 0.05)(F, D)),
        }
    _B_in = _B_setup()

    return {
        "A_x": _A_in["x"],
        "A_k_cache": _A_in["k_cache"],
        "A_v_cache": _A_in["v_cache"],
        "A_wq": _A_in["wq"],
        "A_wo": _A_in["wo"],
        "B_x": _B_in["x"],
        "B_w_r": _B_in["w_r"],
        "B_w_gate": _B_in["w_gate"],
        "B_w_up": _B_in["w_up"],
        "B_w_down": _B_in["w_down"],
    }

def reference(A_x, A_k_cache, A_v_cache, A_wq, A_wo, B_x, B_w_r, B_w_gate, B_w_up, B_w_down):
    def _A_ref(x, k_cache, v_cache, wq, wo):
        B, Sq, D = x.shape
        Hq, Dh = 32, 192
        Hkv, Sk = k_cache.shape[1], k_cache.shape[2]
        W = min(4096, max(256, Sk // 4))
        rep = Hq // Hkv
        q = (lambda x, *d: x.transpose(*d))((x @ wq).reshape(B, Sq, Hq, Dh), 0, 2, 1, 3)
        k = jnp.repeat(k_cache[:, :, Sk - W:, :], rep, axis=1)
        v = jnp.repeat(v_cache[:, :, Sk - W:, :], rep, axis=1)
        scores = jnp.einsum("bhqd,bhkd->bhqk", q, k) * (Dh ** -0.5)
        p = _softmax(scores, axis=-1)
        o = jnp.einsum("bhqk,bhkd->bhqd", p, v)
        return (lambda x, *d: x.transpose(*d))(o, 0, 2, 1, 3).reshape(B, Sq, Hq * Dh) @ wo

    def _B_ref(x, w_r, w_gate, w_up, w_down):
        B, S, D = x.shape
        C = 2
        r = x @ w_r
        idx = jnp.argsort(-r, axis=-1)[:, :C]
        idx_e = jnp.repeat(idx.reshape(B, C, 1), D, axis=2)
        x_sel = jnp.take_along_axis(x, idx_e, axis=1)
        g = _silu(x_sel @ w_gate)
        u = x_sel @ w_up
        y = (g * u) @ w_down
        r_sel = _sigmoid(jnp.take_along_axis(r, idx, axis=1))
        y = y * r_sel.reshape(B, C, 1)
        b_off = (jnp.arange(B) * S).reshape(B, 1)
        flat_idx = (idx + b_off).reshape(B * C)
        zero = (x * 0.0).reshape(B * S, D)
        upd = _scatter_add(zero, flat_idx, y.reshape(B * C, D), axis=0)
        return x + upd.reshape(B, S, D)

    x = A_x
    xn = _layernorm(x, axis=-1)
    s = _A_ref(xn, A_k_cache, A_v_cache, A_wq, A_wo)
    g = _silu(_B_ref(xn, B_w_r, B_w_gate, B_w_up, B_w_down))
    return x + s * g
```

```python
import functools

import jax
import jax.numpy as jnp
import jax.experimental.pallas as pl
import jax.experimental.pallas.tpu as pltpu

f32 = jnp.float32
bf16 = jnp.bfloat16

S = 2048
D = 640
H = 32
DH = 192
SK = 2048
W = 512
F = 1536
NP = H // 2
PW = 2 * DH
CK = 128
NCK = W // CK
LN_EPS = 1e-5
LOG2E = 1.4426950408889634
QSCALE = (DH ** -0.5) * LOG2E

NT_DIMS = (((1,), (1,)), ((), ()))

XC = 512
NXC = S // XC
TB_MID = 2048


def _rb(v):
    return v.astype(bf16).astype(f32)


def _sigmoid(v):
    return 0.5 * jnp.tanh(0.5 * v) + 0.5


def _silu(v):
    h = 0.5 * v
    return h * jnp.tanh(h) + h


def _kernel(x_hbm, kT_hbm, vT_hbm, wq_hbm, wo_hbm, wr_hbm, wg_hbm, wu_hbm, wd_hbm,
            out_hbm,
            x_buf, xn_buf, acc_ref, out_buf,
            wq_buf, wo_buf, kT_buf, vT_buf, kp_ref, woT_ref,
            wr_buf, wg_buf, wu_buf, wd_buf, r_buf, sel_ref,
            sem_x, sem_w, sem_f, sem_o):

    def x_copy(c):
        rows = pl.ds(c * XC if isinstance(c, int) else pl.multiple_of(c * XC, XC), XC)
        return pltpu.make_async_copy(x_hbm.at[rows, :], x_buf.at[rows, :], sem_x.at[c])

    def w_copies(p, slot):
        if isinstance(p, int):
            col, hd = p * PW, 2 * p
        else:
            col, hd = pl.multiple_of(p * PW, 128), 2 * p
        return (
            pltpu.make_async_copy(wq_hbm.at[:, pl.ds(col, PW)], wq_buf.at[slot], sem_w.at[slot, 0]),
            pltpu.make_async_copy(kT_hbm.at[0, pl.ds(hd, 2), :, pl.ds(SK - W, W)], kT_buf.at[slot],
                                  sem_w.at[slot, 1]),
            pltpu.make_async_copy(vT_hbm.at[0, pl.ds(hd, 2), :, pl.ds(SK - W, W)], vT_buf.at[slot],
                                  sem_w.at[slot, 2]),
            pltpu.make_async_copy(wo_hbm.at[pl.ds(col, PW), :], wo_buf.at[slot], sem_w.at[slot, 3]),
        )

    def f_copies():
        return (
            pltpu.make_async_copy(wr_hbm, wr_buf, sem_f.at[0]),
            pltpu.make_async_copy(wg_hbm, wg_buf, sem_f.at[1]),
            pltpu.make_async_copy(wu_hbm, wu_buf, sem_f.at[2]),
            pltpu.make_async_copy(wd_hbm, wd_buf, sem_f.at[3]),
        )

    def o_copy(c):
        rows = pl.ds(c * XC, XC)
        return pltpu.make_async_copy(out_buf.at[rows, :], out_hbm.at[rows, :], sem_o.at[c])

    def prep_k(slot):
        z = jnp.zeros((64, W), bf16)
        kp_ref[0] = jnp.concatenate([kT_buf[slot, 0], z], axis=0).T
        kp_ref[1] = jnp.concatenate([z, kT_buf[slot, 1]], axis=0).T

    def prep_wo(slot):
        woT_ref[...] = wo_buf[slot].T

    def router_lhs():
        wr = wr_buf[...].astype(f32)
        row = jnp.concatenate([wr[k:k + 1, :] for k in range(D // 128)], axis=1)
        return jnp.broadcast_to(row, (16, D)).astype(bf16)

    def layernorm(c):
        rows = pl.ds(pl.multiple_of(c * XC, XC), XC)
        x = x_buf[rows, :].astype(f32)
        mean = jnp.sum(x, axis=1, keepdims=True) * (1.0 / D)
        cen = x - mean
        var = jnp.sum(cen * cen, axis=1, keepdims=True) * (1.0 / D)
        eps = jnp.full((), LN_EPS, bf16).astype(f32)
        den = _rb(jnp.sqrt(_rb(_rb(var) + eps)))
        xn = (_rb(x - _rb(mean)) * (1.0 / den)).astype(bf16)
        xn_buf[rows, :] = xn
        r_buf[:, rows] = _rb(jax.lax.dot_general(router_lhs(), xn, NT_DIMS, preferred_element_type=f32))

    def select_top2():
        r = r_buf[0:8, :]
        idx = jax.lax.broadcasted_iota(jnp.int32, (8, S), 1)
        m1 = jnp.max(r, axis=1, keepdims=True)
        i1 = jnp.min(jnp.where(r == m1, idx, S - 1), axis=1, keepdims=True)
        rest = idx != i1
        r2 = jnp.where(rest, r, -jnp.inf)
        m2 = jnp.max(r2, axis=1, keepdims=True)
        i2 = jnp.min(jnp.where(jnp.logical_and(r2 == m2, rest), idx, S - 1), axis=1, keepdims=True)
        sel_ref[0] = i1[0, 0]
        sel_ref[1] = i2[0, 0]

    def routed_ffn():
        row16 = jax.lax.broadcasted_iota(jnp.int32, (16, 1), 0)
        lane = jax.lax.broadcasted_iota(jnp.int32, (1, 128), 1)
        xrows, rvals = [], []
        for t in range(2):
            i = jnp.clip(sel_ref[t], 0, S - 1)
            base = pl.multiple_of((i // 16) * 16, 16)
            blk = xn_buf[pl.ds(base, 16), :].astype(f32)
            xrows.append(jnp.sum(jnp.where(row16 == i - base, blk, 0.0), axis=0, keepdims=True))
            lbase = pl.multiple_of((i // 128) * 128, 128)
            rblk = r_buf[0:1, pl.ds(lbase, 128)]
            rvals.append(jnp.sum(jnp.where(lane == i - lbase, rblk, 0.0), axis=1, keepdims=True))
        xsel = jnp.where(row16 == 0, xrows[0], jnp.where(row16 == 1, xrows[1], 0.0)).astype(bf16)
        ga = _rb(jnp.dot(xsel, wg_buf[...], preferred_element_type=f32))
        up = _rb(jnp.dot(xsel, wu_buf[...], preferred_element_type=f32))
        hid = (_rb(_silu(ga)) * up).astype(bf16)
        y = _rb(jnp.dot(hid, wd_buf[...], preferred_element_type=f32))
        return [_rb(y[t:t + 1, :] * _rb(_sigmoid(rvals[t]))) for t in range(2)]

    def qproj(slot, start, size):
        xn = xn_buf[pl.ds(start, size), :]
        return (jnp.dot(xn, wq_buf[slot], preferred_element_type=f32) * QSCALE).astype(bf16)

    def scores(q):
        return [jax.lax.dot_general(kp_ref[h], q[:, 128 * h:128 * h + 256], NT_DIMS,
                                    preferred_element_type=f32) for h in range(2)]

    def values(slot, sTs):
        oTs = []
        for h in range(2):
            sT = sTs[h]
            ms, ls, os_ = [], [], []
            for c in range(NCK):
                sc = sT[c * CK:(c + 1) * CK]
                m = jnp.max(sc, axis=0, keepdims=True)
                e = jnp.exp2(sc - m)
                ls.append(jnp.sum(e, axis=0, keepdims=True))
                ms.append(m)
                os_.append(jnp.dot(vT_buf[slot, h, :, c * CK:(c + 1) * CK], e.astype(bf16),
                                   preferred_element_type=f32))
            m = functools.reduce(jnp.maximum, ms)
            al = [jnp.exp2(mc - m) for mc in ms]
            l = functools.reduce(lambda a, b: a + b, [a * b for a, b in zip(al, ls)])
            inv = 1.0 / l
            oT = functools.reduce(lambda a, b: a + b, [(a * inv) * o for a, o in zip(al, os_)])
            oTs.append(oT.astype(bf16))
        oT = jnp.concatenate(oTs, axis=0)
        return jnp.dot(woT_ref[...], oT, preferred_element_type=f32)

    def attention(slot, start, size):
        return values(slot, scores(qproj(slot, start, size)))

    fc = f_copies()
    with jax.named_scope("s0_start"):
        def start_x(c, carry):
            x_copy(c).start()
            return carry
        fc[0].start()
        jax.lax.fori_loop(0, NXC, start_x, 0)
        for cp in w_copies(0, 0):
            cp.start()
        acc_ref[...] = jnp.zeros_like(acc_ref)
        fc[0].wait()

    def ln_step(c, carry):
        x_copy(c).wait()
        layernorm(c)
        return carry

    with jax.named_scope("s1_ln"):
        jax.lax.fori_loop(0, NXC, ln_step, 0)
    with jax.named_scope("s2_top2"):
        for cp in fc[1:]:
            cp.start()
        select_top2()

    def mid(p, carry):
        slot = p % 2
        with jax.named_scope("s4_mid"):
            for cp in w_copies(p, slot):
                cp.wait()
            for cp in w_copies(p + 1, 1 - slot):
                cp.start()
            prep_k(slot)
            prep_wo(slot)
            for j in range(S // TB_MID):
                acc_ref[:, pl.ds(j * TB_MID, TB_MID)] += attention(slot, j * TB_MID, TB_MID)
        return carry

    jax.lax.fori_loop(0, NP - 1, mid, 0)

    last = (NP - 1) % 2
    with jax.named_scope("s6_last"):
        for cp in w_copies(NP - 1, last):
            cp.wait()
        for cp in fc[1:]:
            cp.wait()
        prep_k(last)
        prep_wo(last)
        upds = None
        for c in range(NXC):
            rows = pl.ds(c * XC, XC)
            sTs = scores(qproj(last, c * XC, XC))
            if c == 0:
                upds = routed_ffn()
            sT = acc_ref[:, rows] + values(last, sTs)
            s = sT.T
            tok = c * XC + jax.lax.broadcasted_iota(jnp.int32, (XC, 1), 0)
            upd = jnp.where(tok == sel_ref[0], upds[0], jnp.where(tok == sel_ref[1], upds[1], 0.0))
            g = _silu(_rb(xn_buf[rows, :].astype(f32) + upd))
            out_buf[rows, :] = (x_buf[rows, :].astype(f32) + s * g).astype(bf16)
            o_copy(c).start()
    with jax.named_scope("s7_owait"):
        for c in range(NXC):
            o_copy(c).wait()


@jax.jit
def pallas_recurrent_scan__sliding_block_cached__moe_arch_mod__prompt_kernel(
    A_x: jax.Array,
    A_k_cache: jax.Array,
    A_v_cache: jax.Array,
    A_wq: jax.Array,
    A_wo: jax.Array,
    B_x: jax.Array,
    B_w_r: jax.Array,
    B_w_gate: jax.Array,
    B_w_up: jax.Array,
    B_w_down: jax.Array,
):
    del B_x
    hbm = pl.BlockSpec(memory_space=pl.ANY)
    out = pl.pallas_call(
        _kernel,
        out_shape=jax.ShapeDtypeStruct((S, D), bf16),
        in_specs=[hbm] * 9,
        out_specs=hbm,
        scratch_shapes=[
            pltpu.VMEM((S, D), bf16),
            pltpu.VMEM((S, D), bf16),
            pltpu.VMEM((D, S), f32),
            pltpu.VMEM((S, D), bf16),
            pltpu.VMEM((2, D, PW), bf16),
            pltpu.VMEM((2, PW, D), bf16),
            pltpu.VMEM((2, 2, DH, W), bf16),
            pltpu.VMEM((2, 2, DH, W), bf16),
            pltpu.VMEM((2, W, 256), bf16),
            pltpu.VMEM((D, PW), bf16),
            pltpu.VMEM((D // 128, 128), bf16),
            pltpu.VMEM((D, F), bf16),
            pltpu.VMEM((D, F), bf16),
            pltpu.VMEM((F, D), bf16),
            pltpu.VMEM((16, S), f32),
            pltpu.SMEM((2,), jnp.int32),
            pltpu.SemaphoreType.DMA((NXC,)),
            pltpu.SemaphoreType.DMA((2, 4)),
            pltpu.SemaphoreType.DMA((4,)),
            pltpu.SemaphoreType.DMA((NXC,)),
        ],
        compiler_params=pltpu.CompilerParams(vmem_limit_bytes=120 * 1024 * 1024),
        name="fused_attn_mod",
    )(
        A_x.reshape(S, D),
        jnp.swapaxes(A_k_cache, 2, 3),
        jnp.swapaxes(A_v_cache, 2, 3),
        A_wq,
        A_wo,
        B_w_r.reshape(D // 128, 128),
        B_w_gate,
        B_w_up,
        B_w_down,
    )
    return out.reshape(1, S, D)
```

```python
import functools

import jax
import jax.numpy as jnp
import jax.experimental.pallas as pl
import jax.experimental.pallas.tpu as pltpu

f32 = jnp.float32
bf16 = jnp.bfloat16

S = 2048
D = 640
H = 32
DH = 192
SK = 2048
W = 512
F = 1536
NP = H // 2
PW = 2 * DH
CK = 128
NCK = W // CK
LN_EPS = 1e-5
LOG2E = 1.4426950408889634
QSCALE = (DH ** -0.5) * LOG2E

NT_DIMS = (((1,), (1,)), ((), ()))

XC = 512
NXC = S // XC
OUT_PIECES = ((0, 512), (512, 512), (1024, 512), (1536, 256), (1792, 128), (1920, 128))
TB_MID = 2048


def _rb(v):
    return v.astype(bf16).astype(f32)


def _sigmoid(v):
    return 0.5 * jnp.tanh(0.5 * v) + 0.5


def _silu(v):
    h = 0.5 * v
    return h * jnp.tanh(h) + h


def _kernel(x_hbm, kT_hbm, vT_hbm, wq_hbm, wo_hbm, wr_hbm, wg_hbm, wu_hbm, wd_hbm,
            out_hbm,
            x_buf, xn_buf, acc_ref, out_buf,
            wq_buf, wo_buf, kT_buf, vT_buf, kp_ref, woT_ref,
            wr_buf, wg_buf, wu_buf, wd_buf, q_buf, r_buf,
            sem_x, sem_w, sem_f, sem_o):

    def x_copy(c):
        rows = pl.ds(c * XC if isinstance(c, int) else pl.multiple_of(c * XC, XC), XC)
        return pltpu.make_async_copy(x_hbm.at[rows, :], x_buf.at[rows, :], sem_x.at[c])

    def _col(p):
        return p * PW if isinstance(p, int) else pl.multiple_of(p * PW, 128)

    def wq_copy(p):
        return pltpu.make_async_copy(wq_hbm.at[:, pl.ds(_col(p), PW)], wq_buf.at[p % 2], sem_w.at[p % 2, 0])

    def k_copy(p):
        return pltpu.make_async_copy(kT_hbm.at[0, pl.ds(2 * p, 2), :, pl.ds(SK - W, W)], kT_buf.at[p % 2],
                                     sem_w.at[p % 2, 1])

    def v_copy(p):
        return pltpu.make_async_copy(vT_hbm.at[0, pl.ds(2 * p, 2), :, pl.ds(SK - W, W)], vT_buf.at[p % 2],
                                     sem_w.at[p % 2, 2])

    def wo_copy(p):
        return pltpu.make_async_copy(wo_hbm.at[pl.ds(_col(p), PW), :], wo_buf.at[p % 2], sem_w.at[p % 2, 3])

    def f_copies():
        return (
            pltpu.make_async_copy(wr_hbm, wr_buf, sem_f.at[0]),
            pltpu.make_async_copy(wg_hbm, wg_buf, sem_f.at[1]),
            pltpu.make_async_copy(wu_hbm, wu_buf, sem_f.at[2]),
            pltpu.make_async_copy(wd_hbm, wd_buf, sem_f.at[3]),
        )

    def o_copy(start, size, i):
        rows = pl.ds(start, size)
        return pltpu.make_async_copy(out_buf.at[rows, :], out_hbm.at[rows, :], sem_o.at[i])

    def prep_k(slot):
        z = jnp.zeros((64, W), bf16)
        kp_ref[0] = jnp.concatenate([kT_buf[slot, 0], z], axis=0).T
        kp_ref[1] = jnp.concatenate([z, kT_buf[slot, 1]], axis=0).T

    def prep_wo(slot):
        woT_ref[...] = wo_buf[slot].T

    def _rows(c):
        return pl.ds(c * XC if isinstance(c, int) else pl.multiple_of(c * XC, XC), XC)

    def layernorm_rows(start, size):
        rows = pl.ds(start, size)
        x = x_buf[rows, :].astype(f32)
        mean = jnp.sum(x, axis=1, keepdims=True) * (1.0 / D)
        cen = x - mean
        var = jnp.sum(cen * cen, axis=1, keepdims=True) * (1.0 / D)
        eps = jnp.full((), LN_EPS, bf16).astype(f32)
        den = _rb(jnp.sqrt(_rb(_rb(var) + eps)))
        xn_buf[rows, :] = (_rb(x - _rb(mean)) * (1.0 / den)).astype(bf16)

    def layernorm(c):
        layernorm_rows(c * XC, XC)

    def router_logits(c):
        rows = _rows(c)
        wr = wr_buf[...].astype(f32)
        row = jnp.concatenate([wr[k:k + 1, :] for k in range(D // 128)], axis=1)
        lhs = jnp.broadcast_to(row, (16, D)).astype(bf16)
        r_buf[:, rows] = _rb(jax.lax.dot_general(lhs, xn_buf[rows, :], NT_DIMS, preferred_element_type=f32))

    def select_top2():
        r = r_buf[0:8, :]
        idx = jax.lax.broadcasted_iota(jnp.int32, (8, S), 1)
        m1 = jnp.max(r, axis=1, keepdims=True)
        i1 = jnp.min(jnp.where(r == m1, idx, S - 1), axis=1, keepdims=True)
        rest = idx != i1
        r2 = jnp.where(rest, r, -jnp.inf)
        m2 = jnp.max(r2, axis=1, keepdims=True)
        i2 = jnp.min(jnp.where(jnp.logical_and(r2 == m2, rest), idx, S - 1), axis=1, keepdims=True)
        return (i1[0:1], i2[0:1]), (m1[0:1], m2[0:1])

    def routed_ffn(sel, rvals):
        row16 = jax.lax.broadcasted_iota(jnp.int32, (16, 1), 0)
        xrows, bases, offs = [], [], []
        for t in range(2):
            i = jnp.clip(sel[t][0, 0], 0, S - 1)
            base = pl.multiple_of((i // 16) * 16, 16)
            blk = xn_buf[pl.ds(base, 16), :].astype(f32)
            xrows.append(jnp.sum(jnp.where(row16 == i - base, blk, 0.0), axis=0, keepdims=True))
            bases.append(base)
            offs.append(i - base)
        xsel = jnp.where(row16 == 0, xrows[0], jnp.where(row16 == 1, xrows[1], 0.0)).astype(bf16)
        ga = _rb(jnp.dot(xsel, wg_buf[...], preferred_element_type=f32))
        up = _rb(jnp.dot(xsel, wu_buf[...], preferred_element_type=f32))
        hid = (_rb(_silu(ga)) * up).astype(bf16)
        y = _rb(jnp.dot(hid, wd_buf[...], preferred_element_type=f32))
        for t in range(2):
            upd = _rb(y[t:t + 1, :] * _rb(_sigmoid(rvals[t])))
            blk = xn_buf[pl.ds(bases[t], 16), :].astype(f32)
            xn_buf[pl.ds(bases[t], 16), :] = jnp.where(row16 == offs[t], xrows[t] + upd, blk).astype(bf16)

    def qproj(slot, start, size):
        rows = pl.ds(start, size)
        q_buf[rows, :] = (jnp.dot(xn_buf[rows, :], wq_buf[slot], preferred_element_type=f32) * QSCALE).astype(bf16)

    def score_h(h, start, size):
        return jax.lax.dot_general(kp_ref[h], q_buf[pl.ds(start, size), 128 * h:128 * h + 256], NT_DIMS,
                                   preferred_element_type=f32)

    def scores(start, size):
        return [score_h(h, start, size) for h in range(2)]

    def pv_h(slot, h, sT):
        ms, ls, os_ = [], [], []
        for c in range(NCK):
            sc = sT[c * CK:(c + 1) * CK]
            m = jnp.max(sc, axis=0, keepdims=True)
            e = jnp.exp2(sc - m)
            ls.append(jnp.sum(e, axis=0, keepdims=True))
            ms.append(m)
            os_.append(jnp.dot(vT_buf[slot, h, :, c * CK:(c + 1) * CK], e.astype(bf16),
                               preferred_element_type=f32))
        m = functools.reduce(jnp.maximum, ms)
        al = [jnp.exp2(mc - m) for mc in ms]
        l = functools.reduce(lambda a, b: a + b, [a * b for a, b in zip(al, ls)])
        inv = 1.0 / l
        oT = functools.reduce(lambda a, b: a + b, [(a * inv) * o for a, o in zip(al, os_)])
        return oT.astype(bf16)

    def pv(slot, sTs):
        return jnp.concatenate([pv_h(slot, h, sTs[h]) for h in range(2)], axis=0)

    def outproj(oT):
        return jnp.dot(woT_ref[...], oT, preferred_element_type=f32)

    fc = f_copies()
    with jax.named_scope("s0_start"):
        def start_x(c, carry):
            x_copy(c).start()
            return carry
        fc[0].start()
        jax.lax.fori_loop(0, NXC, start_x, 0)
        wq_copy(0).start()
        k_copy(0).start()
        v_copy(0).start()
        wo_copy(0).start()
        acc_ref[...] = jnp.zeros_like(acc_ref)
        fc[0].wait()

    def ln_step(c, carry):
        x_copy(c).wait()
        layernorm_rows(pl.multiple_of(c * XC, XC), XC)
        router_logits(c)
        return carry

    with jax.named_scope("s1_ln"):
        jax.lax.fori_loop(0, NXC, ln_step, 0)
        for cp in fc[1:]:
            cp.start()

    def mid(p, carry):
        with jax.named_scope("s4_mid"):
            slot = p % 2
            wq_copy(p).wait()
            k_copy(p).wait()
            v_copy(p).wait()
            wo_copy(p).wait()
            wq_copy(p + 1).start()
            k_copy(p + 1).start()
            v_copy(p + 1).start()
            wo_copy(p + 1).start()
            prep_k(slot)
            prep_wo(slot)
            qproj(slot, 0, S)
            acc_ref[...] += outproj(pv(slot, scores(0, S)))
        return carry

    jax.lax.fori_loop(0, NP - 1, mid, 0)

    last = (NP - 1) % 2

    def finalize(start, size, oT):
        rows = pl.ds(start, size)
        s = (acc_ref[:, rows] + outproj(oT)).T
        g = _silu(xn_buf[rows, :].astype(f32))
        out_buf[rows, :] = (x_buf[rows, :].astype(f32) + s * g).astype(bf16)

    with jax.named_scope("s6_last"):
        wq_copy(NP - 1).wait()
        k_copy(NP - 1).wait()
        v_copy(NP - 1).wait()
        wo_copy(NP - 1).wait()
        for cp in fc[1:]:
            cp.wait()
        prep_k(last)
        prep_wo(last)
        sel, rvals = select_top2()
        qproj(last, 0, S)
        sTs = scores(0, S)
        routed_ffn(sel, rvals)
        oT = pv(last, sTs)
        for i, (start, size) in enumerate(OUT_PIECES):
            finalize(start, size, oT[:, start:start + size])
            o_copy(start, size, i).start()
    with jax.named_scope("s7_owait"):
        for i, (start, size) in enumerate(OUT_PIECES):
            o_copy(start, size, i).wait()


@jax.jit
def pallas_recurrent_scan__sliding_block_cached__moe_arch_mod__prompt_kernel(
    A_x: jax.Array,
    A_k_cache: jax.Array,
    A_v_cache: jax.Array,
    A_wq: jax.Array,
    A_wo: jax.Array,
    B_x: jax.Array,
    B_w_r: jax.Array,
    B_w_gate: jax.Array,
    B_w_up: jax.Array,
    B_w_down: jax.Array,
):
    del B_x
    hbm = pl.BlockSpec(memory_space=pl.ANY)
    out = pl.pallas_call(
        _kernel,
        out_shape=jax.ShapeDtypeStruct((S, D), bf16),
        in_specs=[hbm] * 9,
        out_specs=hbm,
        scratch_shapes=[
            pltpu.VMEM((S, D), bf16),
            pltpu.VMEM((S, D), bf16),
            pltpu.VMEM((D, S), f32),
            pltpu.VMEM((S, D), bf16),
            pltpu.VMEM((2, D, PW), bf16),
            pltpu.VMEM((2, PW, D), bf16),
            pltpu.VMEM((2, 2, DH, W), bf16),
            pltpu.VMEM((2, 2, DH, W), bf16),
            pltpu.VMEM((2, W, 256), bf16),
            pltpu.VMEM((D, PW), bf16),
            pltpu.VMEM((D // 128, 128), bf16),
            pltpu.VMEM((D, F), bf16),
            pltpu.VMEM((D, F), bf16),
            pltpu.VMEM((F, D), bf16),
            pltpu.VMEM((S, PW), bf16),
            pltpu.VMEM((16, S), f32),
            pltpu.SemaphoreType.DMA((NXC,)),
            pltpu.SemaphoreType.DMA((2, 4)),
            pltpu.SemaphoreType.DMA((4,)),
            pltpu.SemaphoreType.DMA((len(OUT_PIECES),)),
        ],
        compiler_params=pltpu.CompilerParams(vmem_limit_bytes=120 * 1024 * 1024, disable_bounds_checks=True),
        name="fused_attn_mod",
    )(
        A_x.reshape(S, D),
        jnp.swapaxes(A_k_cache, 2, 3),
        jnp.swapaxes(A_v_cache, 2, 3),
        A_wq,
        A_wo,
        B_w_r.reshape(D // 128, 128),
        B_w_gate,
        B_w_up,
        B_w_down,
    )
    return out.reshape(1, S, D)
```

```python
import functools

import jax
import jax.numpy as jnp
import jax.experimental.pallas as pl
import jax.experimental.pallas.tpu as pltpu

f32 = jnp.float32
bf16 = jnp.bfloat16

S = 2048
D = 640
H = 32
DH = 192
SK = 2048
W = 512
F = 1536
NP = H // 2
PW = 2 * DH
CK = 128
NCK = W // CK
LN_EPS = 1e-5
LOG2E = 1.4426950408889634
QSCALE = (DH ** -0.5) * LOG2E

NT_DIMS = (((1,), (1,)), ((), ()))

XC = 512
NXC = S // XC
OUT_PIECES = ((0, 512), (512, 512), (1024, 512), (1536, 256), (1792, 128), (1920, 128))
LG = 128
TB_MID = 2048


def _rb(v):
    return v.astype(bf16).astype(f32)


def _sigmoid(v):
    return 0.5 * jnp.tanh(0.5 * v) + 0.5


def _silu(v):
    h = 0.5 * v
    return h * jnp.tanh(h) + h


def _kernel(x_hbm, kT_hbm, vT_hbm, wq_hbm, wo_hbm, wr_hbm, wg_hbm, wu_hbm, wd_hbm,
            out_hbm,
            x_buf, xn_buf, acc_ref, out_buf,
            wq_buf, wo_buf, kT_buf, vT_buf, kp_ref, woT_ref,
            wr_buf, wg_buf, wu_buf, wd_buf, q_buf, r_buf,
            sem_x, sem_w, sem_f, sem_o):

    def x_copy(c):
        rows = pl.ds(c * XC if isinstance(c, int) else pl.multiple_of(c * XC, XC), XC)
        return pltpu.make_async_copy(x_hbm.at[rows, :], x_buf.at[rows, :], sem_x.at[c])

    def _col(p):
        return p * PW if isinstance(p, int) else pl.multiple_of(p * PW, 128)

    def wq_copy(p):
        return pltpu.make_async_copy(wq_hbm.at[:, pl.ds(_col(p), PW)], wq_buf.at[p % 2], sem_w.at[p % 2, 0])

    def k_copy(p):
        return pltpu.make_async_copy(kT_hbm.at[0, pl.ds(2 * p, 2), :, pl.ds(SK - W, W)], kT_buf.at[p % 2],
                                     sem_w.at[p % 2, 1])

    def v_copy(p):
        return pltpu.make_async_copy(vT_hbm.at[0, pl.ds(2 * p, 2), :, pl.ds(SK - W, W)], vT_buf.at[p % 2],
                                     sem_w.at[p % 2, 2])

    def wo_copy(p):
        return pltpu.make_async_copy(wo_hbm.at[pl.ds(_col(p), PW), :], wo_buf.at[p % 2], sem_w.at[p % 2, 3])

    def wr_copy():
        return pltpu.make_async_copy(wr_hbm, wr_buf, sem_f.at[0])

    def ffn_copies():
        return (
            pltpu.make_async_copy(wg_hbm, wg_buf, sem_f.at[1]),
            pltpu.make_async_copy(wu_hbm, wu_buf, sem_f.at[2]),
            pltpu.make_async_copy(wd_hbm, wd_buf, sem_f.at[3]),
        )

    def o_copy(start, size, i):
        rows = pl.ds(start, size)
        return pltpu.make_async_copy(out_buf.at[rows, :], out_hbm.at[rows, :], sem_o.at[i])

    def prep_k(slot):
        z = jnp.zeros((64, W), bf16)
        kp_ref[0] = jnp.concatenate([kT_buf[slot, 0], z], axis=0).T
        kp_ref[1] = jnp.concatenate([z, kT_buf[slot, 1]], axis=0).T

    def prep_wo(slot):
        woT_ref[...] = wo_buf[slot].T

    def _rows(c):
        return pl.ds(c * XC if isinstance(c, int) else pl.multiple_of(c * XC, XC), XC)

    def layernorm_rows(start, size):
        rows = pl.ds(start, size)
        x = x_buf[rows, :].astype(f32)
        mean = jnp.sum(x, axis=1, keepdims=True) * (1.0 / D)
        cen = x - mean
        var = jnp.sum(cen * cen, axis=1, keepdims=True) * (1.0 / D)
        eps = jnp.full((), LN_EPS, bf16).astype(f32)
        den = _rb(jnp.sqrt(_rb(_rb(var) + eps)))
        xn_buf[rows, :] = (_rb(x - _rb(mean)) * (1.0 / den)).astype(bf16)

    def layernorm(c):
        layernorm_rows(c * XC, XC)

    def router_logits(c):
        rows = _rows(c)
        wr = wr_buf[...].astype(f32)
        row = jnp.concatenate([wr[k:k + 1, :] for k in range(D // 128)], axis=1)
        lhs = jnp.broadcast_to(row, (16, D)).astype(bf16)
        r_buf[:, rows] = _rb(jax.lax.dot_general(lhs, xn_buf[rows, :], NT_DIMS, preferred_element_type=f32))

    def select_top2():
        r = r_buf[0:8, :]
        idx = jax.lax.broadcasted_iota(jnp.int32, (8, S), 1)
        m1 = jnp.max(r, axis=1, keepdims=True)
        i1 = jnp.min(jnp.where(r == m1, idx, S - 1), axis=1, keepdims=True)
        rest = idx != i1
        r2 = jnp.where(rest, r, -jnp.inf)
        m2 = jnp.max(r2, axis=1, keepdims=True)
        i2 = jnp.min(jnp.where(jnp.logical_and(r2 == m2, rest), idx, S - 1), axis=1, keepdims=True)
        return (i1[0:1], i2[0:1]), (m1[0:1], m2[0:1])

    def routed_ffn(sel, rvals):
        row16 = jax.lax.broadcasted_iota(jnp.int32, (16, 1), 0)
        xrows, bases, offs = [], [], []
        for t in range(2):
            i = jnp.clip(sel[t][0, 0], 0, S - 1)
            base = pl.multiple_of((i // 16) * 16, 16)
            blk = xn_buf[pl.ds(base, 16), :].astype(f32)
            xrows.append(jnp.sum(jnp.where(row16 == i - base, blk, 0.0), axis=0, keepdims=True))
            bases.append(base)
            offs.append(i - base)
        xsel = jnp.where(row16 == 0, xrows[0], jnp.where(row16 == 1, xrows[1], 0.0)).astype(bf16)
        ga = _rb(jnp.dot(xsel, wg_buf[...], preferred_element_type=f32))
        up = _rb(jnp.dot(xsel, wu_buf[...], preferred_element_type=f32))
        hid = (_rb(_silu(ga)) * up).astype(bf16)
        y = _rb(jnp.dot(hid, wd_buf[...], preferred_element_type=f32))
        for t in range(2):
            upd = _rb(y[t:t + 1, :] * _rb(_sigmoid(rvals[t])))
            blk = xn_buf[pl.ds(bases[t], 16), :].astype(f32)
            xn_buf[pl.ds(bases[t], 16), :] = jnp.where(row16 == offs[t], xrows[t] + upd, blk).astype(bf16)

    def qproj(slot, start, size):
        rows = pl.ds(start, size)
        q_buf[rows, :] = (jnp.dot(xn_buf[rows, :], wq_buf[slot], preferred_element_type=f32) * QSCALE).astype(bf16)

    def score_h(h, start, size):
        return jax.lax.dot_general(kp_ref[h], q_buf[pl.ds(start, size), 128 * h:128 * h + 256], NT_DIMS,
                                   preferred_element_type=f32)

    def scores(start, size):
        return [score_h(h, start, size) for h in range(2)]

    def pv_h(slot, h, sT):
        ms, ls, os_ = [], [], []
        for c in range(NCK):
            sc = sT[c * CK:(c + 1) * CK]
            m = jnp.max(sc, axis=0, keepdims=True)
            e = jnp.exp2(sc - m)
            ls.append(jnp.sum(e, axis=0, keepdims=True))
            ms.append(m)
            os_.append(jnp.dot(vT_buf[slot, h, :, c * CK:(c + 1) * CK], e.astype(bf16),
                               preferred_element_type=f32))
        m = functools.reduce(jnp.maximum, ms)
        al = [jnp.exp2(mc - m) for mc in ms]
        l = functools.reduce(lambda a, b: a + b, [a * b for a, b in zip(al, ls)])
        inv = 1.0 / l
        oT = functools.reduce(lambda a, b: a + b, [(a * inv) * o for a, o in zip(al, os_)])
        return oT.astype(bf16)

    def pv(slot, sTs):
        return jnp.concatenate([pv_h(slot, h, sTs[h]) for h in range(2)], axis=0)

    def outproj(oT):
        return jnp.dot(woT_ref[...], oT, preferred_element_type=f32)


    def ordered(cps):
        def body(i, carry):
            for n, cp in enumerate(cps):
                @pl.when(i == n)
                def _():
                    cp.start()
            return carry
        jax.lax.fori_loop(0, len(cps), body, 0)

    with jax.named_scope("s0_start"):
        ordered([x_copy(0), wq_copy(0), wr_copy(), x_copy(1), x_copy(2), x_copy(3), k_copy(0), v_copy(0), wo_copy(0),
                 wq_copy(1), k_copy(1), v_copy(1), wo_copy(1)])
        wq_copy(0).wait()
        wr_copy().wait()

    NG = XC // LG

    def q_rows(rows, xn):
        q_buf[rows, :] = (jnp.dot(xn, wq_buf[0], preferred_element_type=f32) * QSCALE).astype(bf16)

    def ln_step(c, carry):
        x_copy(c).wait()
        wr = wr_buf[...].astype(f32)
        wr_row = jnp.concatenate([wr[k:k + 1, :] for k in range(D // 128)], axis=1)
        wr_lhs = jnp.broadcast_to(wr_row, (16, D)).astype(bf16)
        lag = pl.ds(pl.multiple_of(jnp.maximum(c * XC - LG, 0), LG), LG)
        q_rows(lag, xn_buf[lag, :])
        for g in range(NG):
            rows = pl.ds(pl.multiple_of(c * XC + g * LG, LG), LG)
            x = x_buf[rows, :].astype(f32)
            mean = jnp.sum(x, axis=1, keepdims=True) * (1.0 / D)
            cen = x - mean
            var = jnp.sum(cen * cen, axis=1, keepdims=True) * (1.0 / D)
            eps = jnp.full((), LN_EPS, bf16).astype(f32)
            den = _rb(jnp.sqrt(_rb(_rb(var) + eps)))
            xn = (_rb(x - _rb(mean)) * (1.0 / den)).astype(bf16)
            xn_buf[rows, :] = xn
            if g + 1 < NG:
                q_rows(rows, xn)
            r_buf[:, rows] = _rb(jax.lax.dot_general(wr_lhs, xn, NT_DIMS, preferred_element_type=f32))
        return carry

    xn_buf[0:LG, :] = jnp.zeros((LG, D), bf16)
    with jax.named_scope("s1_ln"):
        jax.lax.fori_loop(0, NXC, ln_step, 0)

    with jax.named_scope("s2_first"):
        k_copy(0).wait()
        v_copy(0).wait()
        wo_copy(0).wait()
        prep_k(0)
        prep_wo(0)
        q_rows(pl.ds(S - LG, LG), xn_buf[S - LG:S, :])
        acc_ref[...] = outproj(pv(0, scores(0, S)))

    def mid(p, carry):
        with jax.named_scope("s4_mid"):
            slot = p % 2
            wq_copy(p).wait()
            k_copy(p).wait()
            v_copy(p).wait()
            wo_copy(p).wait()
            wq_copy(p + 1).start()
            k_copy(p + 1).start()
            v_copy(p + 1).start()
            wo_copy(p + 1).start()

            @pl.when(p == 2)
            def _():
                for cp in ffn_copies():
                    cp.start()

            prep_k(slot)
            prep_wo(slot)
            qproj(slot, 0, S)
            acc_ref[...] += outproj(pv(slot, scores(0, S)))
        return carry

    jax.lax.fori_loop(1, NP - 1, mid, 0)

    last = (NP - 1) % 2

    def finalize(start, size, oT):
        rows = pl.ds(start, size)
        s = (acc_ref[:, rows] + outproj(oT)).T
        g = _silu(xn_buf[rows, :].astype(f32))
        out_buf[rows, :] = (x_buf[rows, :].astype(f32) + s * g).astype(bf16)

    with jax.named_scope("s6_last"):
        wq_copy(NP - 1).wait()
        k_copy(NP - 1).wait()
        v_copy(NP - 1).wait()
        wo_copy(NP - 1).wait()
        for cp in ffn_copies():
            cp.wait()
        prep_k(last)
        prep_wo(last)
        sel, rvals = select_top2()
        qproj(last, 0, S)
        sTs = scores(0, S)
        routed_ffn(sel, rvals)
        oT = pv(last, sTs)
        for i, (start, size) in enumerate(OUT_PIECES):
            finalize(start, size, oT[:, start:start + size])
            o_copy(start, size, i).start()
    with jax.named_scope("s7_owait"):
        for i, (start, size) in enumerate(OUT_PIECES):
            o_copy(start, size, i).wait()


@jax.jit
def pallas_recurrent_scan__sliding_block_cached__moe_arch_mod__prompt_kernel(
    A_x: jax.Array,
    A_k_cache: jax.Array,
    A_v_cache: jax.Array,
    A_wq: jax.Array,
    A_wo: jax.Array,
    B_x: jax.Array,
    B_w_r: jax.Array,
    B_w_gate: jax.Array,
    B_w_up: jax.Array,
    B_w_down: jax.Array,
):
    del B_x
    hbm = pl.BlockSpec(memory_space=pl.ANY)
    out = pl.pallas_call(
        _kernel,
        out_shape=jax.ShapeDtypeStruct((S, D), bf16),
        in_specs=[hbm] * 9,
        out_specs=hbm,
        scratch_shapes=[
            pltpu.VMEM((S, D), bf16),
            pltpu.VMEM((S, D), bf16),
            pltpu.VMEM((D, S), f32),
            pltpu.VMEM((S, D), bf16),
            pltpu.VMEM((2, D, PW), bf16),
            pltpu.VMEM((2, PW, D), bf16),
            pltpu.VMEM((2, 2, DH, W), bf16),
            pltpu.VMEM((2, 2, DH, W), bf16),
            pltpu.VMEM((2, W, 256), bf16),
            pltpu.VMEM((D, PW), bf16),
            pltpu.VMEM((D // 128, 128), bf16),
            pltpu.VMEM((D, F), bf16),
            pltpu.VMEM((D, F), bf16),
            pltpu.VMEM((F, D), bf16),
            pltpu.VMEM((S, PW), bf16),
            pltpu.VMEM((16, S), f32),
            pltpu.SemaphoreType.DMA((NXC,)),
            pltpu.SemaphoreType.DMA((2, 4)),
            pltpu.SemaphoreType.DMA((4,)),
            pltpu.SemaphoreType.DMA((len(OUT_PIECES),)),
        ],
        compiler_params=pltpu.CompilerParams(vmem_limit_bytes=120 * 1024 * 1024, disable_bounds_checks=True),
        name="fused_attn_mod",
    )(
        A_x.reshape(S, D),
        jnp.swapaxes(A_k_cache, 2, 3),
        jnp.swapaxes(A_v_cache, 2, 3),
        A_wq,
        A_wo,
        B_w_r.reshape(D // 128, 128),
        B_w_gate,
        B_w_up,
        B_w_down,
    )
    return out.reshape(1, S, D)
```

```python
import functools

import jax
import jax.numpy as jnp
import jax.experimental.pallas as pl
import jax.experimental.pallas.tpu as pltpu

f32 = jnp.float32
bf16 = jnp.bfloat16

S = 2048
D = 640
H = 32
DH = 192
SK = 2048
W = 512
F = 1536
NP = H // 2
PW = 2 * DH
CK = 128
NCK = W // CK
LN_EPS = 1e-5
LOG2E = 1.4426950408889634
QSCALE = (DH ** -0.5) * LOG2E

NT_DIMS = (((1,), (1,)), ((), ()))

XC = 512
NXC = S // XC
OUT_PIECES = ((0, 512), (512, 512), (1024, 512), (1536, 256), (1792, 128), (1920, 128))
LG = 128


def _rb(v):
    return v.astype(bf16).astype(f32)


def _sigmoid(v):
    return 0.5 * jnp.tanh(0.5 * v) + 0.5


def _silu(v):
    h = 0.5 * v
    return h * jnp.tanh(h) + h


def _kernel(x_hbm, kT_hbm, vT_hbm, wq_hbm, wo_hbm, wr_hbm, wg_hbm, wu_hbm, wd_hbm,
            out_hbm,
            x_buf, xn_buf, acc_ref, out_buf,
            wq_buf, wo_buf, kT_buf, vT_buf, kp_ref, woT_ref,
            wr_buf, wg_buf, wu_buf, wd_buf, q_buf, r_buf, wq0_buf,
            sem_x, sem_w, sem_f, sem_o, sem_q):

    def x_copy(c):
        rows = pl.ds(c * XC if isinstance(c, int) else pl.multiple_of(c * XC, XC), XC)
        return pltpu.make_async_copy(x_hbm.at[rows, :], x_buf.at[rows, :], sem_x.at[c])

    def _col(p):
        return p * PW if isinstance(p, int) else pl.multiple_of(p * PW, 128)

    def wq_copy(p):
        return pltpu.make_async_copy(wq_hbm.at[:, pl.ds(_col(p), PW)], wq_buf.at[p % 2], sem_w.at[p % 2, 0])

    def k_copy(p):
        return pltpu.make_async_copy(kT_hbm.at[0, pl.ds(2 * p, 2), :, pl.ds(SK - W, W)], kT_buf.at[p % 2],
                                     sem_w.at[p % 2, 1])

    def v_copy(p):
        return pltpu.make_async_copy(vT_hbm.at[0, pl.ds(2 * p, 2), :, pl.ds(SK - W, W)], vT_buf.at[p % 2],
                                     sem_w.at[p % 2, 2])

    def wo_copy(p):
        return pltpu.make_async_copy(wo_hbm.at[pl.ds(_col(p), PW), :], wo_buf.at[p % 2], sem_w.at[p % 2, 3])

    def wq0_copy(n):
        return pltpu.make_async_copy(wq_hbm.at[:, pl.ds(n * 128, 128)], wq0_buf.at[n], sem_q.at[n])

    def wr_copy():
        return pltpu.make_async_copy(wr_hbm, wr_buf, sem_f.at[0])

    def ffn_copies():
        return (
            pltpu.make_async_copy(wg_hbm, wg_buf, sem_f.at[1]),
            pltpu.make_async_copy(wu_hbm, wu_buf, sem_f.at[2]),
            pltpu.make_async_copy(wd_hbm, wd_buf, sem_f.at[3]),
        )

    def o_copy(start, size, i):
        rows = pl.ds(start, size)
        return pltpu.make_async_copy(out_buf.at[rows, :], out_hbm.at[rows, :], sem_o.at[i])

    def prep_k(slot):
        z = jnp.zeros((64, W), bf16)
        kp_ref[0] = jnp.concatenate([kT_buf[slot, 0], z], axis=0).T
        kp_ref[1] = jnp.concatenate([z, kT_buf[slot, 1]], axis=0).T

    def prep_wo(slot):
        woT_ref[...] = wo_buf[slot].T

    def select_top2():
        r = r_buf[0:8, :]
        idx = jax.lax.broadcasted_iota(jnp.int32, (8, S), 1)
        m1 = jnp.max(r, axis=1, keepdims=True)
        i1 = jnp.min(jnp.where(r == m1, idx, S - 1), axis=1, keepdims=True)
        rest = idx != i1
        r2 = jnp.where(rest, r, -jnp.inf)
        m2 = jnp.max(r2, axis=1, keepdims=True)
        i2 = jnp.min(jnp.where(jnp.logical_and(r2 == m2, rest), idx, S - 1), axis=1, keepdims=True)
        return (i1[0:1], i2[0:1]), (m1[0:1], m2[0:1])

    def routed_ffn(sel, rvals):
        row16 = jax.lax.broadcasted_iota(jnp.int32, (16, 1), 0)
        xrows, bases, offs = [], [], []
        for t in range(2):
            i = jnp.clip(sel[t][0, 0], 0, S - 1)
            base = pl.multiple_of((i // 16) * 16, 16)
            blk = xn_buf[pl.ds(base, 16), :].astype(f32)
            xrows.append(jnp.sum(jnp.where(row16 == i - base, blk, 0.0), axis=0, keepdims=True))
            bases.append(base)
            offs.append(i - base)
        xsel = jnp.where(row16 == 0, xrows[0], jnp.where(row16 == 1, xrows[1], 0.0)).astype(bf16)
        ga = _rb(jnp.dot(xsel, wg_buf[...], preferred_element_type=f32))
        up = _rb(jnp.dot(xsel, wu_buf[...], preferred_element_type=f32))
        hid = (_rb(_silu(ga)) * up).astype(bf16)
        y = _rb(jnp.dot(hid, wd_buf[...], preferred_element_type=f32))
        for t in range(2):
            upd = _rb(y[t:t + 1, :] * _rb(_sigmoid(rvals[t])))
            blk = xn_buf[pl.ds(bases[t], 16), :].astype(f32)
            xn_buf[pl.ds(bases[t], 16), :] = jnp.where(row16 == offs[t], xrows[t] + upd, blk).astype(bf16)

    def qproj(slot, start, size):
        rows = pl.ds(start, size)
        q_buf[rows, :] = (jnp.dot(xn_buf[rows, :], wq_buf[slot], preferred_element_type=f32) * QSCALE).astype(bf16)

    def score_h(h, start, size):
        return jax.lax.dot_general(kp_ref[h], q_buf[pl.ds(start, size), 128 * h:128 * h + 256], NT_DIMS,
                                   preferred_element_type=f32)

    def scores(start, size):
        return [score_h(h, start, size) for h in range(2)]

    def pv_h(slot, h, sT):
        ms, ls, os_ = [], [], []
        for c in range(NCK):
            sc = sT[c * CK:(c + 1) * CK]
            m = jnp.max(sc, axis=0, keepdims=True)
            e = jnp.exp2(sc - m)
            ls.append(jnp.sum(e, axis=0, keepdims=True))
            ms.append(m)
            os_.append(jnp.dot(vT_buf[slot, h, :, c * CK:(c + 1) * CK], e.astype(bf16),
                               preferred_element_type=f32))
        m = functools.reduce(jnp.maximum, ms)
        al = [jnp.exp2(mc - m) for mc in ms]
        l = functools.reduce(lambda a, b: a + b, [a * b for a, b in zip(al, ls)])
        inv = 1.0 / l
        oT = functools.reduce(lambda a, b: a + b, [(a * inv) * o for a, o in zip(al, os_)])
        return oT.astype(bf16)

    def pv(slot, sTs):
        return jnp.concatenate([pv_h(slot, h, sTs[h]) for h in range(2)], axis=0)

    def outproj(oT):
        return jnp.dot(woT_ref[...], oT, preferred_element_type=f32)


    def ordered(cps):
        def body(i, carry):
            for n, cp in enumerate(cps):
                @pl.when(i == n)
                def _():
                    cp.start()
            return carry
        jax.lax.fori_loop(0, len(cps), body, 0)

    with jax.named_scope("s0_start"):
        ordered([x_copy(0), wq0_copy(0), wq0_copy(1), wq0_copy(2), wr_copy(), x_copy(1), x_copy(2), x_copy(3), k_copy(0), v_copy(0), wo_copy(0),
                 wq_copy(1), k_copy(1), v_copy(1), wo_copy(1)])
        for n in range(3):
            wq0_copy(n).wait()
        wr_copy().wait()

    NG = XC // LG

    def q_rows(rows, xn):
        for n in range(3):
            q_buf[rows, n * 128:(n + 1) * 128] = (
                jnp.dot(xn, wq0_buf[n], preferred_element_type=f32) * QSCALE).astype(bf16)

    def ln_step(c, carry):
        x_copy(c).wait()
        wr = wr_buf[...].astype(f32)
        wr_row = jnp.concatenate([wr[k:k + 1, :] for k in range(D // 128)], axis=1)
        wr_lhs = jnp.broadcast_to(wr_row, (16, D)).astype(bf16)
        eps = jnp.full((), LN_EPS, bf16).astype(f32)
        lag = pl.ds(pl.multiple_of(jnp.maximum(c * XC - LG, 0), LG), LG)
        q_rows(lag, xn_buf[lag, :])
        for g in range(NG):
            rows = pl.ds(pl.multiple_of(c * XC + g * LG, LG), LG)
            x = x_buf[rows, :].astype(f32)
            mean = jnp.sum(x, axis=1, keepdims=True) * (1.0 / D)
            mean_b = _rb(mean)
            cen = x - mean_b
            off = mean - mean_b
            var = jnp.maximum(jnp.sum(cen * cen, axis=1, keepdims=True) * (1.0 / D) - off * off, 0.0)
            ve = _rb(_rb(var) + eps)
            den = _rb(ve * jax.lax.rsqrt(ve))
            inv = pl.reciprocal(den, approx=True)
            inv = inv * (2.0 - den * inv)
            xn = (cen * inv).astype(bf16)
            xn_buf[rows, :] = xn
            if g + 1 < NG:
                q_rows(rows, xn)
            r_buf[:, rows] = _rb(jax.lax.dot_general(wr_lhs, xn, NT_DIMS, preferred_element_type=f32))
        return carry

    xn_buf[0:LG, :] = jnp.zeros((LG, D), bf16)
    with jax.named_scope("s1_ln"):
        jax.lax.fori_loop(0, NXC, ln_step, 0)

    with jax.named_scope("s2_first"):
        k_copy(0).wait()
        v_copy(0).wait()
        wo_copy(0).wait()
        prep_k(0)
        prep_wo(0)
        q_rows(pl.ds(S - LG, LG), xn_buf[S - LG:S, :])
        acc_ref[...] = outproj(pv(0, scores(0, S)))

    def mid(p, carry):
        with jax.named_scope("s4_mid"):
            slot = p % 2
            wq_copy(p).wait()
            k_copy(p).wait()
            v_copy(p).wait()
            wo_copy(p).wait()
            wq_copy(p + 1).start()
            k_copy(p + 1).start()
            v_copy(p + 1).start()
            wo_copy(p + 1).start()

            @pl.when(p == 2)
            def _():
                for cp in ffn_copies():
                    cp.start()

            prep_k(slot)
            prep_wo(slot)
            qproj(slot, 0, S)
            acc_ref[...] += outproj(pv(slot, scores(0, S)))
        return carry

    jax.lax.fori_loop(1, NP - 1, mid, 0)

    last = (NP - 1) % 2

    def finalize(start, size, oT):
        rows = pl.ds(start, size)
        s = (acc_ref[:, rows] + outproj(oT)).T
        g = _silu(xn_buf[rows, :].astype(f32))
        out_buf[rows, :] = (x_buf[rows, :].astype(f32) + s * g).astype(bf16)

    with jax.named_scope("s6_last"):
        wq_copy(NP - 1).wait()
        k_copy(NP - 1).wait()
        v_copy(NP - 1).wait()
        wo_copy(NP - 1).wait()
        for cp in ffn_copies():
            cp.wait()
        prep_k(last)
        prep_wo(last)
        sel, rvals = select_top2()
        qproj(last, 0, S)
        sTs = scores(0, S)
        routed_ffn(sel, rvals)
        oT = pv(last, sTs)
        for i, (start, size) in enumerate(OUT_PIECES):
            finalize(start, size, oT[:, start:start + size])
            o_copy(start, size, i).start()
    with jax.named_scope("s7_owait"):
        for i, (start, size) in enumerate(OUT_PIECES):
            o_copy(start, size, i).wait()


@jax.jit
def pallas_recurrent_scan__sliding_block_cached__moe_arch_mod__prompt_kernel(
    A_x: jax.Array,
    A_k_cache: jax.Array,
    A_v_cache: jax.Array,
    A_wq: jax.Array,
    A_wo: jax.Array,
    B_x: jax.Array,
    B_w_r: jax.Array,
    B_w_gate: jax.Array,
    B_w_up: jax.Array,
    B_w_down: jax.Array,
):
    del B_x
    hbm = pl.BlockSpec(memory_space=pl.ANY)
    out = pl.pallas_call(
        _kernel,
        out_shape=jax.ShapeDtypeStruct((S, D), bf16),
        in_specs=[hbm] * 9,
        out_specs=hbm,
        scratch_shapes=[
            pltpu.VMEM((S, D), bf16),
            pltpu.VMEM((S, D), bf16),
            pltpu.VMEM((D, S), f32),
            pltpu.VMEM((S, D), bf16),
            pltpu.VMEM((2, D, PW), bf16),
            pltpu.VMEM((2, PW, D), bf16),
            pltpu.VMEM((2, 2, DH, W), bf16),
            pltpu.VMEM((2, 2, DH, W), bf16),
            pltpu.VMEM((2, W, 256), bf16),
            pltpu.VMEM((D, PW), bf16),
            pltpu.VMEM((D // 128, 128), bf16),
            pltpu.VMEM((D, F), bf16),
            pltpu.VMEM((D, F), bf16),
            pltpu.VMEM((F, D), bf16),
            pltpu.VMEM((S, PW), bf16),
            pltpu.VMEM((16, S), f32),
            pltpu.VMEM((3, D, 128), bf16),
            pltpu.SemaphoreType.DMA((NXC,)),
            pltpu.SemaphoreType.DMA((2, 4)),
            pltpu.SemaphoreType.DMA((4,)),
            pltpu.SemaphoreType.DMA((len(OUT_PIECES),)),
            pltpu.SemaphoreType.DMA((3,)),
        ],
        compiler_params=pltpu.CompilerParams(vmem_limit_bytes=120 * 1024 * 1024, disable_bounds_checks=True),
        name="fused_attn_mod",
    )(
        A_x.reshape(S, D),
        jnp.swapaxes(A_k_cache, 2, 3),
        jnp.swapaxes(A_v_cache, 2, 3),
        A_wq,
        A_wo,
        B_w_r.reshape(D // 128, 128),
        B_w_gate,
        B_w_up,
        B_w_down,
    )
    return out.reshape(1, S, D)
```

```python
import functools

import jax
import jax.numpy as jnp
import jax.experimental.pallas as pl
import jax.experimental.pallas.tpu as pltpu

f32 = jnp.float32
bf16 = jnp.bfloat16

S = 2048
D = 640
H = 32
DH = 192
SK = 2048
W = 512
F = 1536
NP = H // 2
PW = 2 * DH
CK = 128
NCK = W // CK
LN_EPS = 1e-5
LOG2E = 1.4426950408889634
QSCALE = (DH ** -0.5) * LOG2E

NT_DIMS = (((1,), (1,)), ((), ()))

XC = 512
NXC = S // XC
OUT_PIECES = ((0, 512), (512, 512), (1024, 512), (1536, 256), (1792, 128), (1920, 128))
LG = 128


def _rb(v):
    return v.astype(bf16).astype(f32)


def _sigmoid(v):
    return 0.5 * jnp.tanh(0.5 * v) + 0.5


def _silu(v):
    h = 0.5 * v
    return h * jnp.tanh(h) + h


def _kernel(x_hbm, kT_hbm, vT_hbm, wq_hbm, wo_hbm, wr_hbm, wg_hbm, wu_hbm, wd_hbm,
            out_hbm,
            x_buf, xn_buf, acc_ref, out_buf,
            wq_buf, wo_buf, kT_buf, vT_buf, kp_ref, woT_ref,
            wr_buf, wg_buf, wu_buf, wd_buf, q_buf, r_buf, wq0_buf,
            sem_x, sem_w, sem_f, sem_o, sem_q):

    def x_copy(c):
        rows = pl.ds(c * XC if isinstance(c, int) else pl.multiple_of(c * XC, XC), XC)
        return pltpu.make_async_copy(x_hbm.at[rows, :], x_buf.at[rows, :], sem_x.at[c])

    def _col(p):
        return p * PW if isinstance(p, int) else pl.multiple_of(p * PW, 128)

    def wq_copy(p):
        return pltpu.make_async_copy(wq_hbm.at[:, pl.ds(_col(p), PW)], wq_buf.at[p & 1], sem_w.at[p & 1, 0])

    def k_copy(p):
        return pltpu.make_async_copy(kT_hbm.at[0, pl.ds(2 * p, 2), :, pl.ds(SK - W, W)], kT_buf.at[p & 1],
                                     sem_w.at[p & 1, 1])

    def v_copy(p):
        return pltpu.make_async_copy(vT_hbm.at[0, pl.ds(2 * p, 2), :, pl.ds(SK - W, W)], vT_buf.at[p & 1],
                                     sem_w.at[p & 1, 2])

    def wo_copy(p):
        return pltpu.make_async_copy(wo_hbm.at[pl.ds(_col(p), PW), :], wo_buf.at[p & 1], sem_w.at[p & 1, 3])

    def wq0_copy(n):
        return pltpu.make_async_copy(wq_hbm.at[:, pl.ds(n * 128, 128)], wq0_buf.at[n], sem_q.at[n])

    def wr_copy():
        return pltpu.make_async_copy(wr_hbm, wr_buf, sem_f.at[0])

    def ffn_copies():
        return (
            pltpu.make_async_copy(wg_hbm, wg_buf, sem_f.at[1]),
            pltpu.make_async_copy(wu_hbm, wu_buf, sem_f.at[2]),
            pltpu.make_async_copy(wd_hbm, wd_buf, sem_f.at[3]),
        )

    def o_copy(start, size, i):
        rows = pl.ds(start, size)
        return pltpu.make_async_copy(out_buf.at[rows, :], out_hbm.at[rows, :], sem_o.at[i])

    def prep_k(slot):
        z = jnp.zeros((64, W), bf16)
        kp_ref[0] = jnp.concatenate([kT_buf[slot, 0], z], axis=0).T
        kp_ref[1] = jnp.concatenate([z, kT_buf[slot, 1]], axis=0).T

    def prep_wo(slot):
        woT_ref[...] = wo_buf[slot].T

    def select_top2():
        r = r_buf[0:8, :]
        idx = jax.lax.broadcasted_iota(jnp.int32, (8, S), 1)
        m1 = jnp.max(r, axis=1, keepdims=True)
        i1 = jnp.min(jnp.where(r == m1, idx, S - 1), axis=1, keepdims=True)
        rest = idx != i1
        r2 = jnp.where(rest, r, -jnp.inf)
        m2 = jnp.max(r2, axis=1, keepdims=True)
        i2 = jnp.min(jnp.where(jnp.logical_and(r2 == m2, rest), idx, S - 1), axis=1, keepdims=True)
        return (i1[0:1], i2[0:1]), (m1[0:1], m2[0:1])

    def routed_ffn(sel, rvals):
        row16 = jax.lax.broadcasted_iota(jnp.int32, (16, 1), 0)
        xrows, bases, offs = [], [], []
        for t in range(2):
            i = jnp.clip(sel[t][0, 0], 0, S - 1)
            base = pl.multiple_of((i // 16) * 16, 16)
            blk = xn_buf[pl.ds(base, 16), :].astype(f32)
            xrows.append(jnp.sum(jnp.where(row16 == i - base, blk, 0.0), axis=0, keepdims=True))
            bases.append(base)
            offs.append(i - base)
        xsel = jnp.where(row16 == 0, xrows[0], jnp.where(row16 == 1, xrows[1], 0.0)).astype(bf16)
        ga = _rb(jnp.dot(xsel, wg_buf[...], preferred_element_type=f32))
        up = _rb(jnp.dot(xsel, wu_buf[...], preferred_element_type=f32))
        hid = (_rb(_silu(ga)) * up).astype(bf16)
        y = _rb(jnp.dot(hid, wd_buf[...], preferred_element_type=f32))
        for t in range(2):
            upd = _rb(y[t:t + 1, :] * _rb(_sigmoid(rvals[t])))
            blk = xn_buf[pl.ds(bases[t], 16), :].astype(f32)
            xn_buf[pl.ds(bases[t], 16), :] = jnp.where(row16 == offs[t], xrows[t] + upd, blk).astype(bf16)

    def qproj(slot, start, size):
        rows = pl.ds(start, size)
        q_buf[rows, :] = (jnp.dot(xn_buf[rows, :], wq_buf[slot], preferred_element_type=f32) * QSCALE).astype(bf16)

    def score_h(h, start, size):
        return jax.lax.dot_general(kp_ref[h], q_buf[pl.ds(start, size), 128 * h:128 * h + 256], NT_DIMS,
                                   preferred_element_type=f32)

    def scores(start, size):
        return [score_h(h, start, size) for h in range(2)]

    def pv_h(slot, h, sT):
        ms, ls, os_ = [], [], []
        for c in range(NCK):
            sc = sT[c * CK:(c + 1) * CK]
            m = jnp.max(sc, axis=0, keepdims=True)
            e = jnp.exp2(sc - m)
            ls.append(jnp.sum(e, axis=0, keepdims=True))
            ms.append(m)
            os_.append(jnp.dot(vT_buf[slot, h, :, c * CK:(c + 1) * CK], e.astype(bf16),
                               preferred_element_type=f32))
        m = functools.reduce(jnp.maximum, ms)
        al = [jnp.exp2(mc - m) for mc in ms]
        l = functools.reduce(lambda a, b: a + b, [a * b for a, b in zip(al, ls)])
        inv = 1.0 / l
        oT = functools.reduce(lambda a, b: a + b, [(a * inv) * o for a, o in zip(al, os_)])
        return oT.astype(bf16)

    def pv(slot, sTs):
        return jnp.concatenate([pv_h(slot, h, sTs[h]) for h in range(2)], axis=0)

    def outproj(oT):
        return jnp.dot(woT_ref[...], oT, preferred_element_type=f32)


    def ordered(cps):
        def body(i, carry):
            for n, cp in enumerate(cps):
                @pl.when(i == n)
                def _():
                    cp.start()
            return carry
        jax.lax.fori_loop(0, len(cps), body, 0)

    with jax.named_scope("s0_start"):
        ordered([x_copy(0), wq0_copy(0), wq0_copy(1), wq0_copy(2), wr_copy(), x_copy(1), x_copy(2), x_copy(3), k_copy(0), v_copy(0), wo_copy(0),
                 wq_copy(1), k_copy(1), v_copy(1), wo_copy(1)])
        for n in range(3):
            wq0_copy(n).wait()
        wr_copy().wait()

    NG = XC // LG

    def q_rows(rows, xn):
        for n in range(3):
            q_buf[rows, n * 128:(n + 1) * 128] = (
                jnp.dot(xn, wq0_buf[n], preferred_element_type=f32) * QSCALE).astype(bf16)

    def ln_step(c, carry):
        x_copy(c).wait()
        wr = wr_buf[...].astype(f32)
        wr_row = jnp.concatenate([wr[k:k + 1, :] for k in range(D // 128)], axis=1)
        wr_lhs = jnp.broadcast_to(wr_row, (16, D)).astype(bf16)
        eps = jnp.full((), LN_EPS, bf16).astype(f32)
        lag = pl.ds(pl.multiple_of(jnp.maximum(c * XC - LG, 0), LG), LG)
        q_rows(lag, xn_buf[lag, :])
        for g in range(NG):
            rows = pl.ds(pl.multiple_of(c * XC + g * LG, LG), LG)
            x = x_buf[rows, :].astype(f32)
            mean = jnp.sum(x, axis=1, keepdims=True) * (1.0 / D)
            mean_b = _rb(mean)
            cen = x - mean_b
            off = mean - mean_b
            var = jnp.maximum(jnp.sum(cen * cen, axis=1, keepdims=True) * (1.0 / D) - off * off, 0.0)
            ve = _rb(_rb(var) + eps)
            den = _rb(ve * jax.lax.rsqrt(ve))
            inv = pl.reciprocal(den, approx=True)
            inv = inv * (2.0 - den * inv)
            xn = (cen * inv).astype(bf16)
            xn_buf[rows, :] = xn
            if g + 1 < NG:
                q_rows(rows, xn)
            r_buf[:, rows] = _rb(jax.lax.dot_general(wr_lhs, xn, NT_DIMS, preferred_element_type=f32))
        return carry

    xn_buf[0:LG, :] = jnp.zeros((LG, D), bf16)
    with jax.named_scope("s1_ln"):
        jax.lax.fori_loop(0, NXC, ln_step, 0)

    with jax.named_scope("s2_first"):
        k_copy(0).wait()
        v_copy(0).wait()
        wo_copy(0).wait()
        prep_k(0)
        prep_wo(0)
        q_rows(pl.ds(S - LG, LG), xn_buf[S - LG:S, :])
        acc_ref[...] = outproj(pv(0, scores(0, S)))

    def mid(p, carry):
        with jax.named_scope("s4_mid"):
            slot = p & 1
            wq_copy(p).wait()
            k_copy(p).wait()
            v_copy(p).wait()
            wo_copy(p).wait()
            prep_k(slot)
            prep_wo(slot)
            qproj(slot, 0, S)
            wq_copy(p + 1).start()
            k_copy(p + 1).start()
            v_copy(p + 1).start()
            wo_copy(p + 1).start()
            acc_ref[...] += outproj(pv(slot, scores(0, S)))

            @pl.when(p == 2)
            def _():
                for cp in ffn_copies():
                    cp.start()

        return carry

    jax.lax.fori_loop(1, NP - 1, mid, 0)

    last = (NP - 1) % 2

    def finalize(start, size, oT):
        rows = pl.ds(start, size)
        s = (acc_ref[:, rows] + outproj(oT)).T
        g = _silu(xn_buf[rows, :].astype(f32))
        out_buf[rows, :] = (x_buf[rows, :].astype(f32) + s * g).astype(bf16)

    with jax.named_scope("s6_last"):
        wq_copy(NP - 1).wait()
        k_copy(NP - 1).wait()
        v_copy(NP - 1).wait()
        wo_copy(NP - 1).wait()
        for cp in ffn_copies():
            cp.wait()
        prep_k(last)
        prep_wo(last)
        sel, rvals = select_top2()
        qproj(last, 0, S)
        sTs = scores(0, S)
        routed_ffn(sel, rvals)
        oT = pv(last, sTs)
        for i, (start, size) in enumerate(OUT_PIECES):
            finalize(start, size, oT[:, start:start + size])
            o_copy(start, size, i).start()
    with jax.named_scope("s7_owait"):
        for i, (start, size) in enumerate(OUT_PIECES):
            o_copy(start, size, i).wait()


@jax.jit
def pallas_recurrent_scan__sliding_block_cached__moe_arch_mod__prompt_kernel(
    A_x: jax.Array,
    A_k_cache: jax.Array,
    A_v_cache: jax.Array,
    A_wq: jax.Array,
    A_wo: jax.Array,
    B_x: jax.Array,
    B_w_r: jax.Array,
    B_w_gate: jax.Array,
    B_w_up: jax.Array,
    B_w_down: jax.Array,
):
    del B_x
    hbm = pl.BlockSpec(memory_space=pl.ANY)
    out = pl.pallas_call(
        _kernel,
        out_shape=jax.ShapeDtypeStruct((S, D), bf16),
        in_specs=[hbm] * 9,
        out_specs=hbm,
        scratch_shapes=[
            pltpu.VMEM((S, D), bf16),
            pltpu.VMEM((S, D), bf16),
            pltpu.VMEM((D, S), f32),
            pltpu.VMEM((S, D), bf16),
            pltpu.VMEM((2, D, PW), bf16),
            pltpu.VMEM((2, PW, D), bf16),
            pltpu.VMEM((2, 2, DH, W), bf16),
            pltpu.VMEM((2, 2, DH, W), bf16),
            pltpu.VMEM((2, W, 256), bf16),
            pltpu.VMEM((D, PW), bf16),
            pltpu.VMEM((D // 128, 128), bf16),
            pltpu.VMEM((D, F), bf16),
            pltpu.VMEM((D, F), bf16),
            pltpu.VMEM((F, D), bf16),
            pltpu.VMEM((S, PW), bf16),
            pltpu.VMEM((16, S), f32),
            pltpu.VMEM((3, D, 128), bf16),
            pltpu.SemaphoreType.DMA((NXC,)),
            pltpu.SemaphoreType.DMA((2, 4)),
            pltpu.SemaphoreType.DMA((4,)),
            pltpu.SemaphoreType.DMA((len(OUT_PIECES),)),
            pltpu.SemaphoreType.DMA((3,)),
        ],
        compiler_params=pltpu.CompilerParams(vmem_limit_bytes=120 * 1024 * 1024, disable_bounds_checks=True),
        name="fused_attn_mod",
    )(
        A_x.reshape(S, D),
        jnp.swapaxes(A_k_cache, 2, 3),
        jnp.swapaxes(A_v_cache, 2, 3),
        A_wq,
        A_wo,
        B_w_r.reshape(D // 128, 128),
        B_w_gate,
        B_w_up,
        B_w_down,
    )
    return out.reshape(1, S, D)
```
